```python
import os as _os
_os.environ.setdefault("JAX_PLATFORMS", "cpu")
import jax
import jax.numpy as jnp

def _softmax(x, axis=-1):
    return jax.nn.softmax(x, axis=axis)
def _gelu(x):
    return jax.nn.gelu(x, approximate=True)
def _silu(x):
    return jax.nn.silu(x)
def _sigmoid(x):
    return jax.nn.sigmoid(x)
def _layernorm(x, axis=-1, eps=1e-5):
    m = jnp.mean(x, axis=axis, keepdims=True)
    v = jnp.var(x, axis=axis, keepdims=True)
    return (x - m) / jnp.sqrt(v + eps)
def _scatter_add(tgt, idx, src, axis=0):
    return tgt.at[idx].add(src)
def _segment_sum(src, seg, n):
    return jax.ops.segment_sum(src, seg, n)
class _Rng:
    def __init__(self, key):
        self._k = key
    def _next(self):
        self._k, sub = jax.random.split(self._k)
        return sub
    def normal(self, shape):
        return jax.random.normal(self._next(), shape, dtype=jnp.bfloat16)
    def randint(self, lo, hi, shape):
        return jax.random.randint(self._next(), shape, lo, hi, dtype=jnp.int32)
    def uniform(self, shape, lo=0.0, hi=1.0):
        return jax.random.uniform(self._next(), shape, jnp.bfloat16, lo, hi)
    def permutation(self, n):
        return jax.random.permutation(self._next(), n)


kernel_name = 'parallel_sum__ssm_conv_s5__glu_gated_swiglu__prompt'

def setup_inputs():
    _rng = _Rng(jax.random.key(int.from_bytes(__import__("os").urandom(4), "little")))
    _w = (lambda a: (lambda t: t.astype(jnp.bfloat16) if jnp.issubdtype(t.dtype, jnp.floating) else t)(jnp.asarray(a)))
    def _A_setup():
        B, S, D = 1, 2048, 640
        P = D
        Lambda_re = -0.5 * jnp.exp((lambda *s: _rng.normal(s) * 0.4)(P))
        Lambda_im = (lambda *s: _rng.normal(s) * 0.4)(P) * 1.0
        B_re = (lambda *s: _rng.normal(s) * 0.4)(P, D) * (D ** -0.5)
        B_im = (lambda *s: _rng.normal(s) * 0.4)(P, D) * (D ** -0.5)
        C_re = (lambda *s: _rng.normal(s) * 0.4)(D, P) * (P ** -0.5)
        C_im = (lambda *s: _rng.normal(s) * 0.4)(D, P) * (P ** -0.5)
        log_dt = (lambda *s: _rng.normal(s) * 0.4)(P) * 0.3 - 2.0
        Dskip = (lambda *s: _rng.normal(s) * 0.4)(D)
        return {
            "x": _w((lambda *s: _rng.normal(s) * 0.05)(B, S, D)),
            "Lambda_re": _w(Lambda_re),
            "Lambda_im": _w(Lambda_im),
            "B_re": _w(B_re),
            "B_im": _w(B_im),
            "C_re": _w(C_re),
            "C_im": _w(C_im),
            "log_dt": _w(log_dt),
            "Dskip": _w(Dskip),
        }
    _A_in = _A_setup()

    def _B_setup():
        B, S, D, F = 1, 2048, 640, 1728
        return {
            "x": _w((lambda *s: _rng.normal(s) * 0.05)(B, S, D)),
            "w1": _w((lambda *s: _rng.normal(s) * 0.1)(D, F) * (2.0 / D) ** 0.5),
            "w3": _w((lambda *s: _rng.normal(s) * 0.1)(D, F) * (2.0 / D) ** 0.5),
            "w2": _w((lambda *s: _rng.normal(s) * 0.1)(F, D) * (2.0 / F) ** 0.5),
        }
    _B_in = _B_setup()

    return {
        "A_x": _A_in["x"],
        "A_Lambda_re": _A_in["Lambda_re"],
        "A_Lambda_im": _A_in["Lambda_im"],
        "A_B_re": _A_in["B_re"],
        "A_B_im": _A_in["B_im"],
        "A_C_re": _A_in["C_re"],
        "A_C_im": _A_in["C_im"],
        "A_log_dt": _A_in["log_dt"],
        "A_Dskip": _A_in["Dskip"],
        "B_x": _B_in["x"],
        "B_w1": _B_in["w1"],
        "B_w3": _B_in["w3"],
        "B_w2": _B_in["w2"],
    }

def reference(A_x, A_Lambda_re, A_Lambda_im, A_B_re, A_B_im, A_C_re, A_C_im, A_log_dt, A_Dskip, B_x, B_w1, B_w3, B_w2):
    def _A_ref(x, Lambda_re, Lambda_im, B_re, B_im, C_re, C_im, log_dt, Dskip):
        Bsz, L, H = x.shape
        Lam = Lambda_re + 1j * Lambda_im
        Bmat = B_re + 1j * B_im
        Cmat = C_re + 1j * C_im
        dt = jnp.exp(log_dt)
        Lam_bar = jnp.exp(dt * Lam)
        B_bar = ((Lam_bar - 1.0) / Lam)[:, None] * Bmat
        Bu = jnp.einsum("bld,pd->blp", x + 0j, B_bar)
        h = jnp.zeros_like(Bu[:, 0, :])
        hs = []
        for t in range(L):
            h = Lam_bar[None, :] * h + Bu[:, t, :]
            hs.append(h)
        hseq = jnp.stack(hs, 1)
        y = 2.0 * jnp.einsum("blp,dp->bld", hseq, Cmat).real + x * Dskip[None, None, :]
        return y

    def _B_ref(x, w1, w3, w2):
        gate = jnp.einsum("bsd,df->bsf", x, w1)
        up = jnp.einsum("bsd,df->bsf", x, w3)
        h = _silu(gate) * up
        out = jnp.einsum("bsf,fd->bsd", h, w2)
        return out

    x = A_x
    xn = _layernorm(x, axis=-1)
    return x + _A_ref(xn, A_Lambda_re, A_Lambda_im, A_B_re, A_B_im, A_C_re, A_C_im, A_log_dt, A_Dskip) + _B_ref(xn, B_w1, B_w3, B_w2)
```

```python
import functools
import jax
import jax.numpy as jnp
from jax import lax
import jax.experimental.pallas as pl
import jax.experimental.pallas.tpu as pltpu

S, D, P, F = 2048, 640, 640, 1728
T = 256
NCH = S // T
NSEG = 8
K = T // NSEG
FM = 1664
FL = F - FM
FP = FM + 128
NC = D // 128
NG = P // 128
EPS = 1e-5
XP = K + 1
OP = K + 8
FBLK = ((0, 2), (2, 4), (6, 4), (10, 3))

NT = (((1,), (1,)), ((), ()))
NN = (((1,), (0,)), ((), ()))


def _dot(a, b, dims):
    return lax.dot_general(a, b, dims, preferred_element_type=jnp.float32)


def _cmul(ar, ai, br, bi):
    return ar * br - ai * bi, ar * bi + ai * br


def _silu_mul(g, u):
    return g * jax.nn.sigmoid(g) * u


def _kernel(x_hbm, lre_hbm, lim_hbm, ldt_hbm, dsk_hbm, bre_hbm, bim_hbm, cre_hbm, cim_hbm,
            w1_hbm, w3_hbm, w2_hbm, o_hbm,
            x_v, vecs0, vecs1, vecs2, vecs3, wb, w13, cw, w2s, tab, st, xs, xnb, bu, hs, hf, yacc, stage,
            sem_in, sem_out):
    groups = {}

    def add(g, src, dst):
        if g not in groups:
            groups[g] = (len(groups), [])
        c = pltpu.make_async_copy(src, dst, sem_in.at[groups[g][0]])
        groups[g][1].append(c)
        c.start()

    def rows(ref, a, n):
        return ref.at[pl.ds(a, n)]

    def add_b(g, g0, n):
        add(g, rows(bre_hbm, g0, n), wb.at[pl.ds(g0, n), 0])
        add(g, rows(bim_hbm, g0, n), wb.at[pl.ds(g0, n), 1])

    def add_w(g, t0, nt):
        add(g, rows(w1_hbm, 128 * t0, 128 * nt), rows(w13, 128 * t0, 128 * nt))
        add(g, rows(w3_hbm, 128 * t0, 128 * nt), rows(w13, FM + 128 * t0, 128 * nt))

    add('v', lre_hbm, vecs0)
    add('v', lim_hbm, vecs1)
    add('v', ldt_hbm, vecs2)
    add('v', dsk_hbm, vecs3)
    add('x0', rows(x_hbm, 0, T), rows(x_v, 0, T))
    add('x1', rows(x_hbm, T, T), rows(x_v, T, T))
    add_b('g1', 0, 1)
    add_b('g2', 1, 2)
    add_b('g3', 3, 2)
    add_w('g3', 0, 2)
    add_w('g4', 2, 8)
    add_w('g5', 10, 3)
    add('g5', rows(w1_hbm, FM, FL), rows(w13, 2 * FM, FL))
    add('g5', rows(w3_hbm, FM, FL), rows(w13, 2 * FM + FL, FL))
    add('g5', cre_hbm, cw.at[0])
    add('g5', cim_hbm, cw.at[1])
    add('g5', w2_hbm, rows(w2s, 0, F))
    add('xr', rows(x_hbm, 2 * T, S - 2 * T), rows(x_v, 2 * T, S - 2 * T))

    def wait(g):
        for c in groups[g][1]:
            c.wait()

    def out_copy(i, c):
        return pltpu.make_async_copy(
            stage.at[i, c].reshape(NSEG, OP, 128).at[:, pl.ds(0, K), :],
            o_hbm.at[pl.ds(i * NSEG, NSEG), :, pl.ds(128 * c, 128)],
            sem_out.at[0])

    def tables():
        lre = vecs0[...].astype(jnp.float32).reshape(1, P)
        lim = vecs1[...].astype(jnp.float32).reshape(1, P)
        dt = jnp.exp(vecs2[...].astype(jnp.float32).reshape(1, P)).astype(jnp.bfloat16).astype(jnp.float32)
        mag = jnp.exp(dt * lre)
        ang = dt * lim
        ar = mag * jnp.cos(ang)
        ai = mag * jnp.sin(ang)
        nr = ar - 1.0
        ni = ai
        den = lre * lre + lim * lim
        cr = (nr * lre + ni * lim) / den
        ci = (ni * lre - nr * lim) / den
        tab[0] = jnp.broadcast_to(ar, (8, P))
        tab[1] = jnp.broadcast_to(ai, (8, P))
        pr, pi_ = ar, ai
        k = 1
        while k < K:
            pr, pi_ = _cmul(pr, pi_, pr, pi_)
            k *= 2
        row8 = lax.broadcasted_iota(jnp.int32, (8, P), 0)
        for n, sh in enumerate((1, 2, 4)):
            tab[2 + 2 * n] = jnp.where(row8 >= sh, jnp.broadcast_to(pr, (8, P)), 0.0)
            tab[3 + 2 * n] = jnp.where(row8 >= sh, jnp.broadcast_to(pi_, (8, P)), 0.0)
            pr, pi_ = _cmul(pr, pi_, pr, pi_)
        tab[8] = jnp.broadcast_to(2.0 * cr, (8, P))
        tab[9] = jnp.broadcast_to(-2.0 * ci, (8, P))
        tab[10] = jnp.broadcast_to(vecs3[...].astype(jnp.float32).reshape(1, D), (8, D))

    def xperm(q):
        return jnp.concatenate(
            [jnp.concatenate([xs[q, c, pl.ds((K // 8) * (k % 8) + k // 8, NSEG, stride=XP), :]
                              for k in range(K)], axis=0)
             for c in range(NC)], axis=1)

    def head(q, r0):
        xf = x_v[pl.ds(r0, T), :].astype(jnp.float32)
        for c in range(NC):
            for j in range(NSEG):
                for kh in range(K // 8):
                    xs[q, c, pl.ds(XP * j + kh, 8, stride=K // 8), :] = (
                        xf[K * j + 8 * kh:K * j + 8 * kh + 8, 128 * c:128 * (c + 1)])
        xp = xperm(q)
        m = jnp.mean(xp, axis=-1, keepdims=True)
        xc = xp - m
        v = jnp.mean(xc * xc, axis=-1, keepdims=True)
        xn = xc * lax.rsqrt(v + EPS)
        xnb[q] = xn.astype(jnp.bfloat16)

    def scan(q, g):
        ln = slice(128 * g, 128 * (g + 1))
        cre_ = slice(256 * g, 256 * g + 128)
        cim_ = slice(256 * g + 128, 256 * g + 256)
        lr = tab[0, :, ln]
        li = tab[1, :, ln]
        er = bu[q, 0:8, cre_]
        ei = bu[q, 0:8, cim_]
        for k in range(1, K):
            br = bu[q, 8 * k:8 * k + 8, cre_]
            bi = bu[q, 8 * k:8 * k + 8, cim_]
            er, ei = lr * er - li * ei + br, lr * ei + li * er + bi
        row = lax.broadcasted_iota(jnp.int32, (8, 128), 0)
        zr = pltpu.roll(jnp.where(row == 7, st[0, :, ln], er), 1, 0)
        zi = pltpu.roll(jnp.where(row == 7, st[1, :, ln], ei), 1, 0)
        for n, sh in enumerate((1, 2, 4)):
            mr = tab[2 + 2 * n, :, ln]
            mi = tab[3 + 2 * n, :, ln]
            sr = pltpu.roll(zr, sh, 0)
            si = pltpu.roll(zi, sh, 0)
            zr, zi = zr + (mr * sr - mi * si), zi + (mr * si + mi * sr)
        hr, hi = zr, zi
        ca = tab[8, :, ln]
        cb = tab[9, :, ln]
        for k in range(K):
            br = bu[q, 8 * k:8 * k + 8, cre_]
            bi = bu[q, 8 * k:8 * k + 8, cim_]
            hr, hi = lr * hr - li * hi + br, lr * hi + li * hr + bi
            hs[q, 8 * k:8 * k + 8, ln] = (ca * hr + cb * hi).astype(jnp.bfloat16)
            hs[q, 8 * k:8 * k + 8, P + 128 * g:P + 128 * (g + 1)] = (cb * hr - ca * hi).astype(jnp.bfloat16)
        st[0, :, ln] = hr
        st[1, :, ln] = hi

    def m1(q, g):
        bu[q, :, 256 * g:256 * (g + 1)] = _dot(xnb[q], wb[g].reshape(256, D), NT)

    def m2(q, t0, nt, xb=None):
        xb = xnb[q] if xb is None else xb
        s0, sz = 128 * t0, 128 * nt
        g = _dot(xb, w13[s0:s0 + sz, :], NT)
        u = _dot(xb, w13[FM + s0:FM + s0 + sz, :], NT)
        hf[q, :, s0:s0 + sz] = _silu_mul(g, u).astype(jnp.bfloat16)

    def m2l(q, xb=None):
        xb = xnb[q] if xb is None else xb
        gl = _dot(xb, w13[2 * FM:2 * FM + 128, :], NT)
        ul = pltpu.roll(gl, 64, 1)
        lane = lax.broadcasted_iota(jnp.int32, (T, 128), 1)
        hf[q, :, FM:FP] = jnp.where(lane < FL, _silu_mul(gl, ul), 0.0).astype(jnp.bfloat16)

    def m3a(q):
        base = xperm(q) + xnb[q].astype(jnp.float32) * tab[10][0:1, :]
        yacc[q] = base + _dot(hs[q, :, 0:P], cw[0], NT) + _dot(hs[q, :, P:2 * P], cw[1], NT)

    def m3b(q, i, cols=range(NC)):
        h = hf[q]
        for c in cols:
            y = yacc[q, :, 128 * c:128 * (c + 1)] + _dot(h, w2s[:, 128 * c:128 * (c + 1)], NN)
            for k in range(K):
                stage[i, c, pl.ds(k, NSEG, stride=OP), :] = y[8 * k:8 * k + 8, :]

    def chunk(i):
        head(1, pl.multiple_of(i * T, T))
        m3b(1, i - 1)
        xb = xnb[1]
        bu[1] = _dot(xb, wb[...].reshape(2 * P, D), NT)
        for g in range(NG):
            scan(1, g)
        for (t0, nt) in FBLK:
            m2(1, t0, nt, xb)
        m2l(1, xb)
        m3a(1)

    st[...] = jnp.zeros(st.shape, jnp.float32)
    w2s[F:FP, :] = jnp.zeros((FP - F, D), jnp.bfloat16)
    wait('v')
    tables()
    wait('x0')
    head(0, 0)
    wait('x1')
    head(1, T)
    wait('g1')
    m1(0, 0)
    scan(0, 0)
    m1(1, 0)
    wait('g2')
    scan(1, 0)
    m1(0, 1)
    scan(0, 1)
    m1(1, 1)
    scan(1, 1)
    m1(0, 2)
    scan(0, 2)
    m1(1, 2)
    wait('g3')
    scan(1, 2)
    for g in (3, 4):
        for q in (0, 1):
            m1(q, g)
            scan(q, g)
    for q in (0, 1):
        m2(q, *FBLK[0])
    wait('g4')
    for q in (0, 1):
        m2(q, *FBLK[1])
    for q in (0, 1):
        m2(q, *FBLK[2])
    wait('g5')
    for q in (0, 1):
        m2(q, *FBLK[3])
        m2l(q)
    m3a(0)
    m3b(0, 0)
    m3a(1)
    for c in range(NC):
        out_copy(0, c).start()
    wait('xr')

    def body(i, carry):
        chunk(i)
        for c in range(NC):
            out_copy(i - 1, c).start()
        return carry

    lax.fori_loop(2, NCH, body, 0)

    m3b(1, NCH - 1, range(NC - 1))
    for c in range(NC - 1):
        out_copy(NCH - 1, c).start()
    m3b(1, NCH - 1, (NC - 1,))
    out_copy(NCH - 1, NC - 1).start()
    for i in range(NCH):
        for c in range(NC):
            out_copy(i, c).wait()


@jax.jit
def pallas_parallel_sum__ssm_conv_s5__glu_gated_swiglu__prompt_kernel(
    A_x, A_Lambda_re, A_Lambda_im, A_B_re, A_B_im, A_C_re, A_C_im, A_log_dt, A_Dskip,
    B_x, B_w1, B_w3, B_w2,
):
    x = A_x.reshape(S, D)
    hbm = pl.BlockSpec(memory_space=pl.ANY)
    out = pl.pallas_call(
        _kernel,
        in_specs=[hbm] * 12,
        out_specs=hbm,
        out_shape=jax.ShapeDtypeStruct((S // K, K, D), jnp.float32),
        scratch_shapes=[
            pltpu.VMEM((S, D), jnp.bfloat16),
            pltpu.VMEM((P,), jnp.bfloat16),
            pltpu.VMEM((P,), jnp.bfloat16),
            pltpu.VMEM((P,), jnp.bfloat16),
            pltpu.VMEM((D,), jnp.bfloat16),
            pltpu.VMEM((NG, 2, 128, D), jnp.bfloat16),
            pltpu.VMEM((2 * F, D), jnp.bfloat16),
            pltpu.VMEM((2, D, P), jnp.bfloat16),
            pltpu.VMEM((FP, D), jnp.bfloat16),
            pltpu.VMEM((11, 8, P), jnp.float32),
            pltpu.VMEM((2, 8, P), jnp.float32),
            pltpu.VMEM((2, NC, XP * NSEG, 128), jnp.float32),
            pltpu.VMEM((2, T, D), jnp.bfloat16),
            pltpu.VMEM((2, T, 2 * P), jnp.float32),
            pltpu.VMEM((2, T, 2 * P), jnp.bfloat16),
            pltpu.VMEM((2, T, FP), jnp.bfloat16),
            pltpu.VMEM((2, T, D), jnp.float32),
            pltpu.VMEM((NCH, NC, OP * NSEG, 128), jnp.float32),
            pltpu.SemaphoreType.DMA((9,)),
            pltpu.SemaphoreType.DMA((1,)),
        ],
        compiler_params=pltpu.CompilerParams(
            vmem_limit_bytes=100 * 1024 * 1024,
        ),
    )(x, A_Lambda_re, A_Lambda_im, A_log_dt, A_Dskip,
      A_B_re.reshape(NG, 128, D), A_B_im.reshape(NG, 128, D), A_C_re, A_C_im, B_w1.T, B_w3.T, B_w2)
    return out.reshape(1, S, D)
```

```python
import jax
import jax.numpy as jnp
from jax import lax
import jax.experimental.pallas as pl
import jax.experimental.pallas.tpu as pltpu

S, D, P, F = 2048, 640, 640, 1728
T = 256
NCH = S // T
NSEG = 8
K = T // NSEG
FM = 1664
FL = F - FM
FP = FM + 128
NC = D // 128
NG = P // 128
EPS = 1e-5
XP = K + 1
OP = K + 8
FBLK = ((0, 2), (2, 4), (6, 4), (10, 3))

NT = (((1,), (1,)), ((), ()))
NN = (((1,), (0,)), ((), ()))


def _dot(a, b, dims):
    return lax.dot_general(a, b, dims, preferred_element_type=jnp.float32)


def _cmul(ar, ai, br, bi):
    return ar * br - ai * bi, ar * bi + ai * br


def _silu_mul(g, u):
    return g * jax.nn.sigmoid(g) * u


def _kernel(x_hbm, lre_hbm, lim_hbm, ldt_hbm, dsk_hbm, bre_hbm, bim_hbm, cre_hbm, cim_hbm,
            w1_hbm, w3_hbm, w2_hbm, o_hbm,
            x_v, vecs0, vecs1, vecs2, vecs3, wb, w13, cw, w2s, tab, st, xs, xnb, bu, hs, hf, yacc, stage,
            sem_in, sem_out):
    groups = {}

    def add(g, src, dst):
        if g not in groups:
            groups[g] = (len(groups), [])
        c = pltpu.make_async_copy(src, dst, sem_in.at[groups[g][0]])
        groups[g][1].append(c)
        c.start()

    def rows(ref, a, n):
        return ref.at[pl.ds(a, n)]

    def add_b(g, g0, n):
        add(g, rows(bre_hbm, g0, n), wb.at[pl.ds(g0, n), 0])
        add(g, rows(bim_hbm, g0, n), wb.at[pl.ds(g0, n), 1])

    def add_w(g, t0, nt):
        add(g, rows(w1_hbm, 128 * t0, 128 * nt), rows(w13, 128 * t0, 128 * nt))
        add(g, rows(w3_hbm, 128 * t0, 128 * nt), rows(w13, FM + 128 * t0, 128 * nt))

    add('v', lre_hbm, vecs0)
    add('v', lim_hbm, vecs1)
    add('v', ldt_hbm, vecs2)
    add('v', dsk_hbm, vecs3)
    add('x0', rows(x_hbm, 0, T), rows(x_v, 0, T))
    add('x1', rows(x_hbm, T, T), rows(x_v, T, T))
    add_b('g1', 0, 1)
    add_b('g2', 1, 2)
    add_b('g3', 3, 2)
    add_w('g3', 0, 2)
    add_w('g4', 2, 8)
    add_w('g5', 10, 3)
    add('g5', rows(w1_hbm, FM, FL), rows(w13, 2 * FM, FL))
    add('g5', rows(w3_hbm, FM, FL), rows(w13, 2 * FM + FL, FL))
    add('g5', cre_hbm, cw.at[0])
    add('g5', cim_hbm, cw.at[1])
    add('g5', w2_hbm, rows(w2s, 0, F))
    add('xr', rows(x_hbm, 2 * T, S - 2 * T), rows(x_v, 2 * T, S - 2 * T))

    def wait(g):
        for c in groups[g][1]:
            c.wait()

    def out_copy(i, c):
        return pltpu.make_async_copy(
            stage.at[i, c].reshape(NSEG + 1, OP, 128).at[pl.ds(0, NSEG), pl.ds(0, K), :],
            o_hbm.at[pl.ds(i * NSEG, NSEG), :, pl.ds(128 * c, 128)],
            sem_out.at[0])

    def tables():
        lre = vecs0[...].astype(jnp.float32).reshape(1, P)
        lim = vecs1[...].astype(jnp.float32).reshape(1, P)
        dt = jnp.exp(vecs2[...].astype(jnp.float32).reshape(1, P)).astype(jnp.bfloat16).astype(jnp.float32)
        mag = jnp.exp(dt * lre)
        ang = dt * lim
        ar = mag * jnp.cos(ang)
        ai = mag * jnp.sin(ang)
        nr = ar - 1.0
        ni = ai
        den = lre * lre + lim * lim
        cr = (nr * lre + ni * lim) / den
        ci = (ni * lre - nr * lim) / den
        tab[0] = jnp.broadcast_to(ar, (8, P))
        tab[1] = jnp.broadcast_to(ai, (8, P))
        pr, pi_ = ar, ai
        k = 1
        while k < K:
            pr, pi_ = _cmul(pr, pi_, pr, pi_)
            k *= 2
        row8 = lax.broadcasted_iota(jnp.int32, (8, P), 0)
        for n, sh in enumerate((1, 2, 4)):
            tab[2 + 2 * n] = jnp.where(row8 >= sh, jnp.broadcast_to(pr, (8, P)), 0.0)
            tab[3 + 2 * n] = jnp.where(row8 >= sh, jnp.broadcast_to(pi_, (8, P)), 0.0)
            pr, pi_ = _cmul(pr, pi_, pr, pi_)
        tab[8] = jnp.broadcast_to(2.0 * cr, (8, P))
        tab[9] = jnp.broadcast_to(-2.0 * ci, (8, P))
        tab[10] = jnp.broadcast_to(vecs3[...].astype(jnp.float32).reshape(1, D), (8, D))

    def xperm(q):
        return jnp.concatenate(
            [jnp.concatenate([xs[q, c, pl.ds((K // 8) * (k % 8) + k // 8, NSEG, stride=XP), :]
                              for k in range(K)], axis=0)
             for c in range(NC)], axis=1)

    def head(q, r0):
        xf = x_v[pl.ds(r0, T), :].astype(jnp.float32)
        for c in range(NC):
            for j in range(NSEG):
                for kh in range(K // 8):
                    xs[q, c, pl.ds(XP * j + kh, 8, stride=K // 8), :] = (
                        xf[K * j + 8 * kh:K * j + 8 * kh + 8, 128 * c:128 * (c + 1)])
        xp = xperm(q)
        m = jnp.mean(xp, axis=-1, keepdims=True)
        xc = xp - m
        v = jnp.mean(xc * xc, axis=-1, keepdims=True)
        xn = xc * lax.rsqrt(v + EPS)
        xnb[q] = xn.astype(jnp.bfloat16)

    def scan(q, g):
        ln = slice(128 * g, 128 * (g + 1))
        cre_ = slice(256 * g, 256 * g + 128)
        cim_ = slice(256 * g + 128, 256 * g + 256)
        lr = tab[0, :, ln]
        li = tab[1, :, ln]
        er = bu[q, 0:8, cre_]
        ei = bu[q, 0:8, cim_]
        for k in range(1, K):
            br = bu[q, 8 * k:8 * k + 8, cre_]
            bi = bu[q, 8 * k:8 * k + 8, cim_]
            er, ei = lr * er - li * ei + br, lr * ei + li * er + bi
        row = lax.broadcasted_iota(jnp.int32, (8, 128), 0)
        zr = pltpu.roll(jnp.where(row == 7, st[0, :, ln], er), 1, 0)
        zi = pltpu.roll(jnp.where(row == 7, st[1, :, ln], ei), 1, 0)
        for n, sh in enumerate((1, 2, 4)):
            mr = tab[2 + 2 * n, :, ln]
            mi = tab[3 + 2 * n, :, ln]
            sr = pltpu.roll(zr, sh, 0)
            si = pltpu.roll(zi, sh, 0)
            zr, zi = zr + (mr * sr - mi * si), zi + (mr * si + mi * sr)
        hr, hi = zr, zi
        ca = tab[8, :, ln]
        cb = tab[9, :, ln]
        for k in range(K):
            br = bu[q, 8 * k:8 * k + 8, cre_]
            bi = bu[q, 8 * k:8 * k + 8, cim_]
            hr, hi = lr * hr - li * hi + br, lr * hi + li * hr + bi
            hs[q, 8 * k:8 * k + 8, ln] = (ca * hr + cb * hi).astype(jnp.bfloat16)
            hs[q, 8 * k:8 * k + 8, P + 128 * g:P + 128 * (g + 1)] = (cb * hr - ca * hi).astype(jnp.bfloat16)
        st[0, :, ln] = hr
        st[1, :, ln] = hi

    def m1(q, g):
        bu[q, :, 256 * g:256 * (g + 1)] = _dot(xnb[q], wb[g].reshape(256, D), NT)

    def m2(q, t0, nt, xb=None):
        xb = xnb[q] if xb is None else xb
        s0, sz = 128 * t0, 128 * nt
        g = _dot(xb, w13[s0:s0 + sz, :], NT)
        u = _dot(xb, w13[FM + s0:FM + s0 + sz, :], NT)
        hf[q, :, s0:s0 + sz] = _silu_mul(g, u).astype(jnp.bfloat16)

    def m2l(q, xb=None):
        xb = xnb[q] if xb is None else xb
        gl = _dot(xb, w13[2 * FM:2 * FM + 128, :], NT)
        ul = pltpu.roll(gl, 64, 1)
        lane = lax.broadcasted_iota(jnp.int32, (T, 128), 1)
        hf[q, :, FM:FP] = jnp.where(lane < FL, _silu_mul(gl, ul), 0.0).astype(jnp.bfloat16)

    def m3a(q):
        base = xperm(q) + xnb[q].astype(jnp.float32) * tab[10][0:1, :]
        yacc[q] = base + _dot(hs[q, :, 0:P], cw[0], NT) + _dot(hs[q, :, P:2 * P], cw[1], NT)

    def m3b(q, i, cols=range(NC)):
        h = hf[q]
        for c in cols:
            y = yacc[q, :, 128 * c:128 * (c + 1)] + _dot(h, w2s[:, 128 * c:128 * (c + 1)], NN)
            for k in range(K):
                stage[i, c, pl.ds(k, NSEG, stride=OP), :] = y[8 * k:8 * k + 8, :]

    def chunk(i):
        head(1, pl.multiple_of(i * T, T))
        m3b(1, i - 1)
        xb = xnb[1]
        bu[1] = _dot(xb, wb[...].reshape(2 * P, D), NT)
        for g in range(NG):
            scan(1, g)
        for (t0, nt) in FBLK:
            m2(1, t0, nt, xb)
        m2l(1, xb)
        m3a(1)

    st[...] = jnp.zeros(st.shape, jnp.float32)
    wait('v')
    tables()
    wait('x0')
    head(0, 0)
    wait('x1')
    head(1, T)
    wait('g1')
    m1(0, 0)
    scan(0, 0)
    m1(1, 0)
    wait('g2')
    scan(1, 0)
    m1(0, 1)
    scan(0, 1)
    m1(1, 1)
    scan(1, 1)
    m1(0, 2)
    scan(0, 2)
    m1(1, 2)
    wait('g3')
    scan(1, 2)
    for g in (3, 4):
        for q in (0, 1):
            m1(q, g)
            scan(q, g)
    for q in (0, 1):
        m2(q, *FBLK[0])
    wait('g4')
    for q in (0, 1):
        m2(q, *FBLK[1])
    for q in (0, 1):
        m2(q, *FBLK[2])
    wait('g5')
    w2s[F:FP, :] = jnp.zeros((FP - F, D), jnp.bfloat16)
    for q in (0, 1):
        m2(q, *FBLK[3])
        m2l(q)
    m3a(0)
    m3b(0, 0)
    m3a(1)
    for c in range(NC):
        out_copy(0, c).start()
    wait('xr')

    def body(i, carry):
        chunk(i)
        for c in range(NC):
            out_copy(i - 1, c).start()
        return carry

    lax.fori_loop(2, NCH, body, 0)

    m3b(1, NCH - 1, range(NC - 1))
    for c in range(NC - 1):
        out_copy(NCH - 1, c).start()
    c = NC - 1
    for r0 in (0, T // 2):
        y = (yacc[1, r0:r0 + T // 2, 128 * c:128 * (c + 1)]
             + _dot(hf[1, r0:r0 + T // 2, :], w2s[:, 128 * c:128 * (c + 1)], NN))
        for k in range(K // 2):
            stage[NCH - 1, c, pl.ds(r0 // 8 + k, NSEG, stride=OP), :] = y[8 * k:8 * k + 8, :]
    out_copy(NCH - 1, NC - 1).start()
    for i in range(NCH):
        for c in range(NC):
            out_copy(i, c).wait()


def _compiler_params():
    limit = 100 * 1024 * 1024
    try:
        return pltpu.CompilerParams(vmem_limit_bytes=limit, disable_semaphore_checks=True)
    except TypeError:
        return pltpu.CompilerParams(vmem_limit_bytes=limit)


@jax.jit
def pallas_parallel_sum__ssm_conv_s5__glu_gated_swiglu__prompt_kernel(
    A_x: jax.Array,
    A_Lambda_re: jax.Array,
    A_Lambda_im: jax.Array,
    A_B_re: jax.Array,
    A_B_im: jax.Array,
    A_C_re: jax.Array,
    A_C_im: jax.Array,
    A_log_dt: jax.Array,
    A_Dskip: jax.Array,
    B_x: jax.Array,
    B_w1: jax.Array,
    B_w3: jax.Array,
    B_w2: jax.Array,
):
    x = A_x.reshape(S, D)
    hbm = pl.BlockSpec(memory_space=pl.ANY)
    out = pl.pallas_call(
        _kernel,
        in_specs=[hbm] * 12,
        out_specs=hbm,
        out_shape=jax.ShapeDtypeStruct((S // K, K, D), jnp.float32),
        scratch_shapes=[
            pltpu.VMEM((S, D), jnp.bfloat16),
            pltpu.VMEM((P,), jnp.bfloat16),
            pltpu.VMEM((P,), jnp.bfloat16),
            pltpu.VMEM((P,), jnp.bfloat16),
            pltpu.VMEM((D,), jnp.bfloat16),
            pltpu.VMEM((NG, 2, 128, D), jnp.bfloat16),
            pltpu.VMEM((2 * F, D), jnp.bfloat16),
            pltpu.VMEM((2, D, P), jnp.bfloat16),
            pltpu.VMEM((FP, D), jnp.bfloat16),
            pltpu.VMEM((11, 8, P), jnp.float32),
            pltpu.VMEM((2, 8, P), jnp.float32),
            pltpu.VMEM((2, NC, 296, 128), jnp.float32),
            pltpu.VMEM((2, T, D), jnp.bfloat16),
            pltpu.VMEM((2, T, 2 * P), jnp.float32),
            pltpu.VMEM((2, T, 2 * P), jnp.bfloat16),
            pltpu.VMEM((2, T, FP), jnp.bfloat16),
            pltpu.VMEM((2, T, D), jnp.float32),
            pltpu.VMEM((NCH, NC, OP * (NSEG + 1), 128), jnp.float32),
            pltpu.SemaphoreType.DMA((9,)),
            pltpu.SemaphoreType.DMA((1,)),
        ],
        compiler_params=_compiler_params(),
    )(x, A_Lambda_re, A_Lambda_im, A_log_dt, A_Dskip,
      A_B_re.reshape(NG, 128, D), A_B_im.reshape(NG, 128, D), A_C_re, A_C_im, B_w1.T, B_w3.T, B_w2)
    return out.reshape(1, S, D)
```
